```python
import os as _os
_os.environ.setdefault("JAX_PLATFORMS", "cpu")
import jax
import jax.numpy as jnp

def _softmax(x, axis=-1):
    return jax.nn.softmax(x, axis=axis)
def _gelu(x):
    return jax.nn.gelu(x, approximate=True)
def _silu(x):
    return jax.nn.silu(x)
def _sigmoid(x):
    return jax.nn.sigmoid(x)
def _layernorm(x, axis=-1, eps=1e-5):
    m = jnp.mean(x, axis=axis, keepdims=True)
    v = jnp.var(x, axis=axis, keepdims=True)
    return (x - m) / jnp.sqrt(v + eps)
def _scatter_add(tgt, idx, src, axis=0):
    return tgt.at[idx].add(src)
def _segment_sum(src, seg, n):
    return jax.ops.segment_sum(src, seg, n)
class _Rng:
    def __init__(self, key):
        self._k = key
    def _next(self):
        self._k, sub = jax.random.split(self._k)
        return sub
    def normal(self, shape):
        return jax.random.normal(self._next(), shape, dtype=jnp.bfloat16)
    def randint(self, lo, hi, shape):
        return jax.random.randint(self._next(), shape, lo, hi, dtype=jnp.int32)
    def uniform(self, shape, lo=0.0, hi=1.0):
        return jax.random.uniform(self._next(), shape, jnp.bfloat16, lo, hi)
    def permutation(self, n):
        return jax.random.permutation(self._next(), n)


kernel_name = 'sequential_preLN__compressed_kv_cla__dense_activation_mish__decode'

def setup_inputs():
    _rng = _Rng(jax.random.key(int.from_bytes(__import__("os").urandom(4), "little")))
    _w = (lambda a: (lambda t: t.astype(jnp.bfloat16) if jnp.issubdtype(t.dtype, jnp.floating) else t)(jnp.asarray(a)))
    def _A_setup():
        B, H, Sq, Sk, D, M = 1, 32, 1, 8192, 128, 512
        Dc = 4 * D
        return {
            "x": _w((lambda *s: _rng.normal(s) * 0.05)(B, Sq, M)),
            "c_kv": _w((lambda *s: _rng.normal(s) * 0.8)(B, Sk, Dc)),
            "w_q": _w((lambda *s: _rng.normal(s) * 0.8)(M, H, D) * (M ** -0.5)),
            "w_uk": _w((lambda *s: _rng.normal(s) * 0.8)(Dc, H, D) * (Dc ** -0.5)),
            "w_uv": _w((lambda *s: _rng.normal(s) * 0.8)(Dc, H, D) * (Dc ** -0.5)),
            "w_o": _w((lambda *s: _rng.normal(s) * 0.8)(H, D, M) * ((H * D) ** -0.5)),
        }
    _A_in = _A_setup()

    def _B_setup():
        B, S, D, F = 1, 1, 512, 1376
        return {
            "x": _w((lambda *s: _rng.normal(s) * 0.05)(B, S, D)),
            "w1": _w((lambda *s: _rng.normal(s) * 0.2)(D, F) * (D ** -0.5)),
            "b1": _w((lambda *s: _rng.normal(s) * 0.05)(F)),
            "w2": _w((lambda *s: _rng.normal(s) * 0.05)(F, D) * (F ** -0.5)),
        }
    _B_in = _B_setup()

    return {
        "A_x": _A_in["x"],
        "A_c_kv": _A_in["c_kv"],
        "A_w_q": _A_in["w_q"],
        "A_w_uk": _A_in["w_uk"],
        "A_w_uv": _A_in["w_uv"],
        "A_w_o": _A_in["w_o"],
        "B_x": _B_in["x"],
        "B_w1": _B_in["w1"],
        "B_b1": _B_in["b1"],
        "B_w2": _B_in["w2"],
    }

def reference(A_x, A_c_kv, A_w_q, A_w_uk, A_w_uv, A_w_o, B_x, B_w1, B_b1, B_w2):
    def _A_ref(x, c_kv, w_q, w_uk, w_uv, w_o):
        B, Sq, M = x.shape[0], x.shape[1], x.shape[2]
        Sk = c_kv.shape[1]
        H, D = w_q.shape[1], w_q.shape[2]
        q = jnp.einsum("bqm,mhd->bhqd", x, w_q)
        k = jnp.einsum("bkc,chd->bhkd", c_kv, w_uk)
        v = jnp.einsum("bkc,chd->bhkd", c_kv, w_uv)
        scores = jnp.einsum("bhqd,bhkd->bhqk", q, k) * (D ** -0.5)
        off = Sk - Sq
        qi = jnp.arange(Sq)[:, None]
        kj = jnp.arange(Sk)[None, :]
        cmask = kj <= (qi + off)
        scores = jnp.where(cmask[None, None], scores, -1e9)
        p = _softmax(scores, axis=-1)
        ctx = jnp.einsum("bhqk,bhkd->bhqd", p, v)
        return jnp.einsum("bhqd,hdm->bqm", ctx, w_o)

    def _B_ref(x, w1, b1, w2):
        h = jnp.einsum("bsd,df->bsf", x, w1) + b1
        sp = jnp.log1p(jnp.exp(-jnp.abs(h))) + jnp.where(h > 0, h, jnp.zeros_like(h))
        act = h * jnp.tanh(sp)
        return jnp.einsum("bsf,fd->bsd", act, w2)

    x = A_x
    h = x + _A_ref(_layernorm(x, axis=-1), A_c_kv, A_w_q, A_w_uk, A_w_uv, A_w_o)
    h2 = h + _B_ref(_layernorm(h, axis=-1), B_w1, B_b1, B_w2)
    return h2
```

```python
import functools

import jax
import jax.numpy as jnp
from jax import lax
from jax.experimental import pallas as pl
from jax.experimental.pallas import tpu as pltpu

H, D, M, DC, SK, F = 32, 128, 512, 512, 8192, 1376
NKV = 4
BF = jnp.bfloat16
F32 = jnp.float32
NT = (((1,), (1,)), ((), ()))
SCOPES = False


def _scope(n):
    import contextlib
    return jax.named_scope(n) if SCOPES else contextlib.nullcontext()


def _ln(v):
    m = jnp.mean(v, axis=-1, keepdims=True)
    c = v - m
    var = jnp.mean(c * c, axis=-1, keepdims=True)
    return c / jnp.sqrt(var + 1e-5)


def _kernel(x_hbm, ckv_hbm, wq_hbm, wuk_hbm, wuv_hbm, wo_hbm, w1t_hbm, b1_hbm, w2_hbm, o_ref,
            x_v, ckv_v, wq_v, wuk_v, wuv_v, wo_v, w1t_v, b1_v, w2_v, a_v, sems):
    kc = SK // NKV
    cp_x = pltpu.make_async_copy(x_hbm, x_v, sems.at[0])
    cp_b1 = pltpu.make_async_copy(b1_hbm, b1_v, sems.at[1])
    cp_wq = pltpu.make_async_copy(wq_hbm, wq_v, sems.at[2])
    cp_wuk = pltpu.make_async_copy(wuk_hbm, wuk_v, sems.at[3])
    cp_wuv = pltpu.make_async_copy(wuv_hbm, wuv_v, sems.at[4])
    cp_wo = pltpu.make_async_copy(wo_hbm, wo_v, sems.at[5])
    cp_w1 = pltpu.make_async_copy(w1t_hbm, w1t_v, sems.at[6])
    cp_w2 = pltpu.make_async_copy(w2_hbm, w2_v, sems.at[7])
    cp_kv = [pltpu.make_async_copy(ckv_hbm.at[pl.ds(i * kc, kc)], ckv_v.at[pl.ds(i * kc, kc)], sems.at[8 + i])
             for i in range(NKV)]
    cp_x.start()
    cp_wq.start()
    cp_wuk.start()
    for c in cp_kv:
        c.start()
    cp_wuv.start()
    cp_wo.start()
    cp_b1.start()
    cp_w1.start()
    cp_w2.start()

    lane = lax.broadcasted_iota(jnp.int32, (H, 128), 1)
    row = lax.broadcasted_iota(jnp.int32, (H, 128), 0)
    diag = (lane % H) == row
    r128 = lax.broadcasted_iota(jnp.int32, (128, 128), 0)
    l128 = lax.broadcasted_iota(jnp.int32, (128, 128), 1)
    efix = ((r128 % 4) == (l128 // H)).astype(BF)
    gfix = ((r128 // H) == (l128 % 4)).astype(BF)

    def expand(cm):
        for b in range(4):
            cb = cm[:, 128 * b:128 * (b + 1)]
            lhs = jnp.concatenate([jnp.where((lane // 4) == t, cb, jnp.zeros_like(cb)) for t in range(32)], axis=0)
            e = jnp.dot(lhs, efix, preferred_element_type=F32)
            for t in range(32):
                et = e[32 * t:32 * (t + 1), :]
                a_v[:, pl.ds(128 * (32 * b + t), 128)] = jnp.where(diag, et, 0.0).astype(BF)

    cp_x.wait()
    x = x_v[...].astype(F32)
    xn = _ln(x).astype(BF)
    with _scope("expand1"):
        expand(jnp.broadcast_to(xn, (H, M)))
    with _scope("wait_wq"):
        cp_wq.wait()
    with _scope("mm_wq"):
        q = jnp.dot(a_v[...], wq_v[...], preferred_element_type=F32)
        qb = q.astype(BF)
    with _scope("wait_wuk"):
        cp_wuk.wait()
    with _scope("mm_wuk"):
        qabs = []
        for b in range(4):
            r = lax.dot_general(qb, wuk_v[pl.ds(4096 * b, 4096), :], NT, preferred_element_type=F32)
            lhs = jnp.concatenate(
                [jnp.where(diag, r[:, 128 * t:128 * (t + 1)], 0.0).astype(BF) for t in range(32)], axis=0)
            s = jnp.dot(lhs, gfix, preferred_element_type=F32)
            acc = jnp.zeros((H, 128), F32)
            for t in range(32):
                acc = jnp.where((lane // 4) == t, s[32 * t:32 * (t + 1), :], acc)
            qabs.append(acc)
        qa = (jnp.concatenate(qabs, axis=1) * (D ** -0.5)).astype(BF)
    m_i = jnp.full((H, 1), -jnp.inf, F32)
    l_i = jnp.zeros((H, 1), F32)
    acc = jnp.zeros((H, DC), F32)
    for i in range(NKV):
        with _scope("wait_kv"):
            cp_kv[i].wait()
        with _scope("attn"):
            kv = ckv_v[pl.ds(i * kc, kc), :]
            s = lax.dot_general(qa, kv, NT, preferred_element_type=F32)
            m_new = jnp.maximum(m_i, jnp.max(s, axis=-1, keepdims=True))
            alpha = jnp.exp(m_i - m_new)
            p = jnp.exp(s - m_new)
            l_i = alpha * l_i + jnp.sum(p, axis=-1, keepdims=True)
            acc = alpha * acc + jnp.dot(p.astype(BF), kv, preferred_element_type=F32)
            m_i = m_new
    with _scope("expand5"):
        cc = (acc / l_i).astype(BF)
        expand(cc)
    with _scope("wait_wuv"):
        cp_wuv.wait()
    with _scope("mm_wuv"):
        ctx = jnp.dot(a_v[...], wuv_v[...], preferred_element_type=F32).astype(BF)
        row16 = lax.broadcasted_iota(jnp.int32, (16, 128), 0)
        z = jnp.concatenate(
            [jnp.where(row16 == (h % 16), ctx[16 * (h // 16):16 * (h // 16) + 16, :], jnp.zeros((16, 128), BF))
             for h in range(H)], axis=1)
    with _scope("wait_wo"):
        cp_wo.wait()
    with _scope("mm_wo"):
        o = jnp.dot(z, wo_v[...], preferred_element_type=F32)
        hres = x + jnp.sum(o, axis=0, keepdims=True)
        hn = jnp.broadcast_to(_ln(hres).astype(BF), (16, M))
    with _scope("wait_w1"):
        cp_w1.wait()
        cp_b1.wait()
    with _scope("mm_w1"):
        u = lax.dot_general(hn, w1t_v[...], NT, preferred_element_type=F32) + b1_v[...].astype(F32).reshape(1, F)
        sp = jnp.log1p(jnp.exp(-jnp.abs(u))) + jnp.maximum(u, 0.0)
        act = (u * jnp.tanh(sp)).astype(BF)
    with _scope("wait_w2"):
        cp_w2.wait()
    with _scope("mm_w2"):
        y = jnp.dot(act, w2_v[...], preferred_element_type=F32)
        o_ref[...] = (hres + y[0:1, :]).astype(BF)


@jax.jit
def pallas_sequential_preLN__compressed_kv_cla__dense_activation_mish__decode_kernel(A_x, A_c_kv, A_w_q, A_w_uk, A_w_uv, A_w_o, B_x, B_w1, B_b1, B_w2):
    del B_x
    any_spec = pl.BlockSpec(memory_space=pl.ANY)
    out = pl.pallas_call(
        _kernel,
        out_shape=jax.ShapeDtypeStruct((1, M), BF),
        in_specs=[any_spec] * 9,
        out_specs=pl.BlockSpec(memory_space=pltpu.VMEM),
        scratch_shapes=[
            pltpu.VMEM((1, M), BF),
            pltpu.VMEM((SK, DC), BF),
            pltpu.VMEM((M * H, D), BF),
            pltpu.VMEM((DC * H, D), BF),
            pltpu.VMEM((DC * H, D), BF),
            pltpu.VMEM((H * D, M), BF),
            pltpu.VMEM((F, M), BF),
            pltpu.VMEM((F,), BF),
            pltpu.VMEM((F, M), BF),
            pltpu.VMEM((H, DC * H), BF),
            pltpu.SemaphoreType.DMA((8 + NKV,)),
        ],
        compiler_params=pltpu.CompilerParams(vmem_limit_bytes=64 << 20),
    )(A_x.reshape(1, M), A_c_kv.reshape(SK, DC), A_w_q.reshape(M * H, D), A_w_uk.reshape(DC * H, D),
      A_w_uv.reshape(DC * H, D), A_w_o.reshape(H * D, M), B_w1.T, B_b1, B_w2)
    return out.reshape(1, 1, M)
```

```python
import jax
import jax.numpy as jnp
from jax import lax
from jax.experimental import pallas as pl
from jax.experimental.pallas import tpu as pltpu

H, D, M, DC, SK, F = 32, 128, 512, 512, 8192, 1376
NC = 4
W2_BOUNDS = (0, 896, 1216, F)
BF = jnp.bfloat16
F32 = jnp.float32
NT = (((1,), (1,)), ((), ()))


def _ln(v):
    m = jnp.mean(v, axis=-1, keepdims=True)
    c = v - m
    var = jnp.mean(c * c, axis=-1, keepdims=True)
    return c / jnp.sqrt(var + 1e-5)


def _kernel(x_hbm, ckv_hbm, wq_hbm, wuk_hbm, wuv_hbm, wo_hbm, w1t_hbm, b1_hbm, w2_hbm, o_ref,
            x_v, ckv_v, wq_v, wuk_v, wuv_v, wo_v, w1t_v, b1_v, w2_v, a_v, sems):
    w2b = W2_BOUNDS
    cp_wq = pltpu.make_async_copy(wq_hbm, wq_v, sems.at[0])
    cp_x = pltpu.make_async_copy(x_hbm, x_v, sems.at[0])
    cp_wuk = pltpu.make_async_copy(wuk_hbm, wuk_v, sems.at[1])
    cp_kv = pltpu.make_async_copy(ckv_hbm, ckv_v, sems.at[2])
    cp_wuv = pltpu.make_async_copy(wuv_hbm, wuv_v, sems.at[0])
    cp_wo = pltpu.make_async_copy(wo_hbm, wo_v, sems.at[1])
    cp_b1 = pltpu.make_async_copy(b1_hbm, b1_v, sems.at[2])
    cp_w1 = pltpu.make_async_copy(w1t_hbm, w1t_v, sems.at[2])
    cp_w2 = [pltpu.make_async_copy(w2_hbm.at[pl.ds(w2b[i], w2b[i + 1] - w2b[i])],
                                   w2_v.at[pl.ds(w2b[i], w2b[i + 1] - w2b[i])], sems.at[i])
             for i in range(3)]
    cp_wq.start()
    cp_x.start()
    cp_wuk.start()
    cp_kv.start()

    lane = lax.broadcasted_iota(jnp.int32, (H, 128), 1)
    row = lax.broadcasted_iota(jnp.int32, (H, 128), 0)
    diag = (lane % H) == row
    r128 = lax.broadcasted_iota(jnp.int32, (128, 128), 0)
    l128 = lax.broadcasted_iota(jnp.int32, (128, 128), 1)
    efix = ((r128 % 4) == (l128 // H)).astype(BF)
    gfix = ((r128 // H) == (l128 % 4)).astype(BF)

    def expand(cm):
        for b in range(4):
            cb = cm[:, 128 * b:128 * (b + 1)]
            lhs = jnp.concatenate(
                [jnp.where((lane // 4) == t, cb, jnp.zeros_like(cb)) for t in range(32)], axis=0)
            e = jnp.dot(lhs, efix, preferred_element_type=F32)
            for t in range(32):
                et = e[32 * t:32 * (t + 1), :]
                a_v[:, pl.ds(128 * (32 * b + t), 128)] = jnp.where(diag, et, 0.0).astype(BF)

    cp_x.wait()
    cp_wq.wait()
    cp_wuv.start()
    x = x_v[...].astype(F32)
    xn = _ln(x).astype(BF)
    expand(jnp.broadcast_to(xn, (H, M)))
    qb = jnp.dot(a_v[...], wq_v[...], preferred_element_type=F32).astype(BF)

    cp_wuk.wait()
    cp_wo.start()
    qabs = []
    for b in range(4):
        r = lax.dot_general(qb, wuk_v[pl.ds(4096 * b, 4096), :], NT,
                            preferred_element_type=F32) * (D ** -0.5)
        lhs = jnp.concatenate(
            [jnp.where(diag, r[:, 128 * t:128 * (t + 1)], 0.0).astype(BF) for t in range(32)], axis=0)
        s = jnp.dot(lhs, gfix, preferred_element_type=F32)
        acc = jnp.zeros((H, 128), F32)
        for t in range(32):
            acc = jnp.where((lane // 4) == t, s[32 * t:32 * (t + 1), :], acc)
        qabs.append(acc)
    qa = jnp.concatenate(qabs, axis=1).astype(BF)

    cp_kv.wait()
    cp_b1.start()
    cp_w1.start()
    m_i = jnp.full((H, 1), -jnp.inf, F32)
    l_i = jnp.zeros((H, 1), F32)
    acc = jnp.zeros((H, DC), F32)
    kcc = SK // NC
    for i in range(NC):
        kv = ckv_v[pl.ds(i * kcc, kcc), :]
        s = lax.dot_general(qa, kv, NT, preferred_element_type=F32)
        m_new = jnp.maximum(m_i, jnp.max(s, axis=-1, keepdims=True))
        alpha = jnp.exp(m_i - m_new)
        p = jnp.exp(s - m_new)
        l_i = alpha * l_i + jnp.sum(p, axis=-1, keepdims=True)
        acc = alpha * acc + jnp.dot(p.astype(BF), kv, preferred_element_type=F32)
        m_i = m_new
    expand((acc / l_i).astype(BF))

    cp_wuv.wait()
    cp_w2[0].start()
    ctx = jnp.dot(a_v[...], wuv_v[...], preferred_element_type=F32).astype(BF)
    row16 = lax.broadcasted_iota(jnp.int32, (16, 128), 0)
    z = jnp.concatenate(
        [jnp.where(row16 == (h % 16), ctx[16 * (h // 16):16 * (h // 16) + 16, :], jnp.zeros((16, 128), BF))
         for h in range(H)], axis=1)

    cp_wo.wait()
    cp_w2[1].start()
    o = jnp.dot(z, wo_v[...], preferred_element_type=F32)
    hres = x + jnp.sum(o, axis=0, keepdims=True)
    hn = jnp.broadcast_to(_ln(hres).astype(BF), (16, M))

    cp_w1.wait()
    cp_b1.wait()
    cp_w2[2].start()
    u = lax.dot_general(hn, w1t_v[...], NT, preferred_element_type=F32) + b1_v[...].astype(F32).reshape(1, F)
    sp = jnp.log1p(jnp.exp(-jnp.abs(u))) + jnp.maximum(u, 0.0)
    act = (u * jnp.tanh(sp)).astype(BF)

    r0 = w2b[2]
    nr = F - r0
    npad = (-nr) % 128
    actf = act[0:8, r0:].astype(F32)
    if npad:
        actf = jnp.concatenate([actf, jnp.zeros((8, npad), F32)], axis=1)
    actb = jnp.concatenate(
        [jnp.transpose(jnp.broadcast_to(actf[0:1, 128 * j:128 * (j + 1)], (128, 128)))
         for j in range((nr + npad) // 128)], axis=0)[:nr]

    y = hres
    for i in range(2):
        cp_w2[i].wait()
        y = y + jnp.dot(act[:, w2b[i]:w2b[i + 1]], w2_v[pl.ds(w2b[i], w2b[i + 1] - w2b[i]), :],
                        preferred_element_type=F32)[0:1, :]
    cp_w2[2].wait()
    wt = w2_v[pl.ds(r0, nr), :].astype(F32)
    parts = [jnp.sum(wt[:, 128 * n:128 * (n + 1)] * actb, axis=0, keepdims=True) for n in range(M // 128)]
    y = y + jnp.concatenate(parts, axis=1)
    o_ref[...] = y.astype(BF)


@jax.jit
def pallas_sequential_preLN__compressed_kv_cla__dense_activation_mish__decode_kernel(
    A_x: jax.Array,
    A_c_kv: jax.Array,
    A_w_q: jax.Array,
    A_w_uk: jax.Array,
    A_w_uv: jax.Array,
    A_w_o: jax.Array,
    B_x: jax.Array,
    B_w1: jax.Array,
    B_b1: jax.Array,
    B_w2: jax.Array,
):
    del B_x
    any_spec = pl.BlockSpec(memory_space=pl.ANY)
    out = pl.pallas_call(
        _kernel,
        out_shape=jax.ShapeDtypeStruct((1, M), BF),
        in_specs=[any_spec] * 9,
        out_specs=pl.BlockSpec(memory_space=pltpu.VMEM),
        scratch_shapes=[
            pltpu.VMEM((1, M), BF),
            pltpu.VMEM((SK, DC), BF),
            pltpu.VMEM((M * H, D), BF),
            pltpu.VMEM((DC * H, D), BF),
            pltpu.VMEM((DC * H, D), BF),
            pltpu.VMEM((H * D, M), BF),
            pltpu.VMEM((F, M), BF),
            pltpu.VMEM((F,), BF),
            pltpu.VMEM((F, M), BF),
            pltpu.VMEM((H, DC * H), BF),
            pltpu.SemaphoreType.DMA((3,)),
        ],
        compiler_params=pltpu.CompilerParams(vmem_limit_bytes=64 << 20),
    )(A_x.reshape(1, M), A_c_kv.reshape(SK, DC), A_w_q.reshape(M * H, D), A_w_uk.reshape(DC * H, D),
      A_w_uv.reshape(DC * H, D), A_w_o.reshape(H * D, M), B_w1.T, B_b1, B_w2)
    return out.reshape(1, 1, M)
```
